```python
import os as _os
_os.environ.setdefault('JAX_PLATFORMS', 'cpu')
import jax
import jax.numpy as jnp

def _softmax(x, axis=-1):
    return jax.nn.softmax(x, axis=axis)

def _gelu(x):
    return jax.nn.gelu(x, approximate=True)

def _silu(x):
    return jax.nn.silu(x)

def _sigmoid(x):
    return jax.nn.sigmoid(x)

def _layernorm(x, axis=-1, eps=1e-05):
    m = jnp.mean(x, axis=axis, keepdims=True)
    v = jnp.var(x, axis=axis, keepdims=True)
    return (x - m) / jnp.sqrt(v + eps)

def _scatter_add(tgt, idx, src, axis=0):
    return tgt.at[idx].add(src)

def _segment_sum(src, seg, n):
    return jax.ops.segment_sum(src, seg, n)

class _Rng:

    def __init__(self, key):
        self._k = key

    def _next(self):
        self._k, sub = jax.random.split(self._k)
        return sub

    def normal(self, shape):
        return jax.random.normal(self._next(), shape, dtype=jnp.bfloat16)

    def randint(self, lo, hi, shape):
        return jax.random.randint(self._next(), shape, lo, hi, dtype=jnp.int32)

    def uniform(self, shape, lo=0.0, hi=1.0):
        return jax.random.uniform(self._next(), shape, jnp.bfloat16, lo, hi)

    def permutation(self, n):
        return jax.random.permutation(self._next(), n)
kernel_name = 'adaLN_cond__mha_block_cached__geglu_ffn__prompt'

def setup_inputs():
    _rng = _Rng(jax.random.key(int.from_bytes(__import__("os").urandom(4), "little")))
    _w = lambda a: (lambda t: t.astype(jnp.bfloat16) if jnp.issubdtype(t.dtype, jnp.floating) else t)(jnp.asarray(a))

    def _A_setup():
        B, Sq, D = (1, 2048, 512)
        H, Sk, Dh = (32, 2048, 128)
        return {'x': _w((lambda *s: _rng.normal(s) * 0.05)(B, Sq, D)), 'k_cache': _w((lambda *s: _rng.normal(s) * 3.2)(B, H, Sk, Dh)), 'v_cache': _w((lambda *s: _rng.normal(s) * 0.4)(B, H, Sk, Dh)), 'wq': _w((lambda *s: _rng.normal(s) * 1.6)(D, H * Dh) * D ** (-0.5)), 'wo': _w((lambda *s: _rng.normal(s) * 0.4)(H * Dh, D) * (H * Dh) ** (-0.5))}
    _A_in = _A_setup()

    def _B_setup():
        B, S, D, F = (1, 2048, 512, 1792)
        return {'x': _w((lambda *s: _rng.normal(s) * 0.05)(B, S, D)), 'w_gate': _w((lambda *s: _rng.normal(s) * 0.05)(D, F)), 'w_up': _w((lambda *s: _rng.normal(s) * 0.05)(D, F)), 'w_down': _w((lambda *s: _rng.normal(s) * 0.05)(F, D))}
    _B_in = _B_setup()
    return {'A_x': _A_in['x'], 'A_k_cache': _A_in['k_cache'], 'A_v_cache': _A_in['v_cache'], 'A_wq': _A_in['wq'], 'A_wo': _A_in['wo'], 'B_x': _B_in['x'], 'B_w_gate': _B_in['w_gate'], 'B_w_up': _B_in['w_up'], 'B_w_down': _B_in['w_down'], 'c': _w((lambda *s: _rng.normal(s) * 0.05)(1, 512) * 8.0), 'w_mod': _w((lambda *s: _rng.normal(s) * 0.05)(512, 6 * 512) * 512 ** (-0.5) * 8.0)}

def reference(A_x, A_k_cache, A_v_cache, A_wq, A_wo, B_x, B_w_gate, B_w_up, B_w_down, c, w_mod):

    def _A_ref(x, k_cache, v_cache, wq, wo):
        B, Sq, D = x.shape
        H, Dh = (32, 128)
        q = (lambda x, *d: x.transpose(*d))((x @ wq).reshape(B, Sq, H, Dh), 0, 2, 1, 3)
        scores = jnp.einsum('bhqd,bhkd->bhqk', q, k_cache) * Dh ** (-0.5)
        p = _softmax(scores, axis=-1)
        o = jnp.einsum('bhqk,bhkd->bhqd', p, v_cache)
        return (lambda x, *d: x.transpose(*d))(o, 0, 2, 1, 3).reshape(B, Sq, H * Dh) @ wo

    def _B_ref(x, w_gate, w_up, w_down):
        return _gelu(x @ w_gate) * (x @ w_up) @ w_down
    x = A_x
    mod = (_silu(c) @ w_mod).reshape(c.shape[0], 6, 1, -1)
    sa, ca, ga, sb, cb, gb = (mod[:, 0].copy(), mod[:, 1].copy(), mod[:, 2].copy(), mod[:, 3].copy(), mod[:, 4].copy(), mod[:, 5].copy())
    h = _layernorm(x, axis=-1) * (1 + ca) + sa
    x = x + ga * _A_ref(h, A_k_cache, A_v_cache, A_wq, A_wo)
    h = _layernorm(x, axis=-1) * (1 + cb) + sb
    x = x + gb * _B_ref(h, B_w_gate, B_w_up, B_w_down)
    return x
```

```python
import functools
import math

import jax
import jax.numpy as jnp
from jax import lax
import jax.experimental.pallas as pl
import jax.experimental.pallas.tpu as pltpu

_NT = (((1,), (1,)), ((), ()))
S, D, H, DH, SK, F = 2048, 512, 32, 128, 2048, 1792


def _ln_mod(x, scale1, shift):
    m = jnp.mean(x, axis=-1, keepdims=True)
    xc = x - m
    v = jnp.mean(xc * xc, axis=-1, keepdims=True)
    return xc * lax.rsqrt(v + 1e-5) * scale1 + shift


def _gelu(x):
    return 0.5 * x * (1.0 + jnp.tanh(0.7978845608028654 * (x + 0.044715 * (x * x * x))))


def _make(G, KGA, KGB, FSQ, FC, LSQ, ffn_mode, scopes):
    NG = H // G
    qscale = (DH ** -0.5) * math.log2(math.e)

    def scope(name):
        import contextlib
        return jax.named_scope(name) if scopes else contextlib.nullcontext()

    def kernel(c_ref, x_hbm, k_hbm, v_hbm, wq_hbm, wo_hbm, wg_hbm, wu_hbm, wd_hbm, wmod_hbm, out_hbm,
               x_v, h_v, o_v, s_v, m_v, k0_v, wq0_v, k_v, v_v, wq_v, wo_v, wg_v, wu_v, wd_v, wmod_v, mod_v,
               x1_v, h2_v, out_v,
               sem_misc, sem_k, sem_v, sem_q, sem_out):
        cp_wm0 = pltpu.make_async_copy(wmod_hbm.at[:, pl.ds(0, 2 * D)], wmod_v.at[:, pl.ds(0, 2 * D)], sem_misc.at[0])
        cp_wm1 = pltpu.make_async_copy(wmod_hbm.at[:, pl.ds(2 * D, 4 * D)], wmod_v.at[:, pl.ds(2 * D, 4 * D)], sem_misc.at[1])
        cp_x = pltpu.make_async_copy(x_hbm, x_v, sem_misc.at[2])
        cp_wo = pltpu.make_async_copy(wo_hbm, wo_v, sem_misc.at[3])
        cp_wg = pltpu.make_async_copy(wg_hbm, wg_v, sem_misc.at[4])
        cp_wu = pltpu.make_async_copy(wu_hbm, wu_v, sem_misc.at[5])
        cp_wd = pltpu.make_async_copy(wd_hbm, wd_v, sem_misc.at[6])
        cp_k0 = pltpu.make_async_copy(k_hbm.at[0], k0_v, sem_misc.at[7])
        cp_q0 = pltpu.make_async_copy(wq_hbm.at[:, pl.ds(0, DH)], wq0_v, sem_misc.at[8])

        def kq_start(g):
            return jnp.minimum(g * G + 1, H - G)

        def cp_chunk(g):
            slot = g & 1
            h0 = kq_start(g)
            return (
                pltpu.make_async_copy(v_hbm.at[pl.ds(g * G, G)], v_v.at[slot], sem_v.at[slot]),
                pltpu.make_async_copy(k_hbm.at[pl.ds(h0, G)], k_v.at[slot], sem_k.at[slot]),
                pltpu.make_async_copy(wq_hbm.at[:, pl.ds(pl.multiple_of(h0 * DH, DH), G * DH)], wq_v.at[slot], sem_q.at[slot]),
            )

        with scope("P0"):
            cp_wm0.start()
            cp_x.start()
            cp_q0.start()
            cp_k0.start()

            c = c_ref[...].astype(jnp.float32)
            sc = jnp.broadcast_to(c * jax.nn.sigmoid(c), (16, D)).astype(jnp.bfloat16)
            cp_wm0.wait()
            mod_v[:, 0:2 * D] = jnp.dot(sc, wmod_v[:, 0:2 * D], preferred_element_type=jnp.float32)

            for cp in cp_chunk(0):
                cp.start()
            cp_x.wait()

        sa = mod_v[0:1, 0:D]
        ca1 = 1.0 + mod_v[0:1, D:2 * D]

        def ln_body(i, carry):
            rows = pl.ds(pl.multiple_of(i * LSQ, LSQ), LSQ)
            h_v[rows, :] = _ln_mod(x_v[rows, :].astype(jnp.float32), ca1, sa).astype(jnp.bfloat16)
            return carry

        with scope("P1"):
            lax.fori_loop(0, S // LSQ, ln_body, 0)

        def stage_q(wq):
            q = jnp.dot(h_v[...], wq, preferred_element_type=jnp.float32)
            return (q * qscale).astype(jnp.bfloat16)

        def stage_a(q, kref):
            mx = None
            for g in range(SK // KGA):
                s = lax.dot_general(q, kref[g * KGA:(g + 1) * KGA, :], _NT, preferred_element_type=jnp.float32)
                s_v[:, g * KGA:(g + 1) * KGA] = s
                for j in range(KGA // 128):
                    sj = s[:, j * 128:(j + 1) * 128]
                    mx = sj if mx is None else jnp.maximum(mx, sj)
            m_v[...] = mx

        def stage_b(hd, vref):
            o = None
            l = None
            mm = jnp.broadcast_to(jnp.max(m_v[...], axis=-1, keepdims=True), (S, 128))
            mrep = jnp.concatenate([mm] * (KGB // 128), axis=-1)
            for g in range(SK // KGB):
                p = jnp.exp2(s_v[:, g * KGB:(g + 1) * KGB] - mrep)
                gl = p[:, 0:128]
                for j in range(1, KGB // 128):
                    gl = gl + p[:, j * 128:(j + 1) * 128]
                l = gl if l is None else l + gl
                oo = jnp.dot(p.astype(jnp.bfloat16), vref[g * KGB:(g + 1) * KGB, :], preferred_element_type=jnp.float32)
                o = oo if o is None else o + oo
            lsum = jnp.sum(l, axis=-1, keepdims=True)
            o_v[hd] = (o * (1.0 / lsum)).astype(jnp.bfloat16)

        with scope("P2"):
            cp_q0.wait()
            cp_k0.wait()
            stage_a(stage_q(wq0_v[...]), k0_v)

        cp_wm1.start()
        cp_wo.start()
        cp_wg.start()
        cp_wu.start()
        cp_wd.start()

        def group_body(g, carry):
            for cp in cp_chunk(g):
                cp.wait()

            @pl.when(g + 1 < NG)
            def _():
                for cp in cp_chunk(g + 1):
                    cp.start()

            slot = g & 1
            off = g * G + 1 - kq_start(g)

            def head_body(j, carry):
                ja = j + off
                q = stage_q(wq_v[slot, :, pl.ds(pl.multiple_of(ja * DH, DH), DH)])
                stage_b(g * G + j, v_v.at[slot, j])
                stage_a(q, k_v.at[slot, ja])
                return carry
            lax.fori_loop(0, jnp.where(g == NG - 1, G - 1, G), head_body, 0)
            return carry

        with scope("P3"):
            lax.fori_loop(0, NG, group_body, 0)
        with scope("P4"):
            cp_wm1.wait()
            mod_v[:, 2 * D:6 * D] = jnp.dot(sc, wmod_v[:, 2 * D:6 * D], preferred_element_type=jnp.float32)
            stage_b(H - 1, v_v.at[(NG - 1) & 1, G - 1])

        cp_wo.wait()
        cp_wg.wait()
        cp_wu.wait()
        cp_wd.wait()

        def cp_out(i):
            rows = pl.ds(pl.multiple_of(i * FSQ, FSQ), FSQ)
            return pltpu.make_async_copy(out_v.at[rows, :], out_hbm.at[rows, :], sem_out.at[i])

        def stage_c(i):
            ga = mod_v[0:1, 2 * D:3 * D]
            sb = mod_v[0:1, 3 * D:4 * D]
            cb1 = 1.0 + mod_v[0:1, 4 * D:5 * D]
            rows = pl.ds(pl.multiple_of(i * FSQ, FSQ), FSQ)
            ocat = jnp.concatenate([o_v[hh, rows, :] for hh in range(H)], axis=-1)
            a = jnp.dot(ocat, wo_v[...], preferred_element_type=jnp.float32)
            x1 = x_v[rows, :].astype(jnp.float32) + ga * a
            h2 = _ln_mod(x1, cb1, sb).astype(jnp.bfloat16)
            return x1, h2

        def stage_d(i, x1, h2):
            gb = mod_v[0:1, 5 * D:6 * D]
            rows = pl.ds(pl.multiple_of(i * FSQ, FSQ), FSQ)
            y = None
            for f in range(F // FC):
                cols = slice(f * FC, (f + 1) * FC)
                g = jnp.dot(h2, wg_v[:, cols], preferred_element_type=jnp.float32)
                u = jnp.dot(h2, wu_v[:, cols], preferred_element_type=jnp.float32)
                act = (_gelu(g) * u).astype(jnp.bfloat16)
                yy = jnp.dot(act, wd_v[cols, :], preferred_element_type=jnp.float32)
                y = yy if y is None else y + yy
            out_v[rows, :] = (x1 + gb * y).astype(out_v.dtype)
            cp_out(i).start()

        nf = S // FSQ
        with scope("P5"):
            if ffn_mode == 0:
                def ffn_body(i, carry):
                    x1, h2 = stage_c(i)
                    stage_d(i, x1, h2)
                    return carry
                lax.fori_loop(0, nf, ffn_body, 0)
            elif ffn_mode == 1:
                x1, h2 = stage_c(0)
                x1_v[...] = x1
                h2_v[...] = h2

                def ffn_body(i, carry):
                    x1c = x1_v[...]
                    h2c = h2_v[...]
                    x1n, h2n = stage_c(i + 1)
                    x1_v[...] = x1n
                    h2_v[...] = h2n
                    stage_d(i, x1c, h2c)
                    return carry
                lax.fori_loop(0, nf - 1, ffn_body, 0)
                stage_d(nf - 1, x1_v[...], h2_v[...])
            elif ffn_mode == 2:
                def ffn_body(i, carry):
                    x1a, h2a = stage_c(2 * i)
                    x1b, h2b = stage_c(2 * i + 1)
                    stage_d(2 * i, x1a, h2a)
                    stage_d(2 * i + 1, x1b, h2b)
                    return carry
                lax.fori_loop(0, nf // 2, ffn_body, 0)
            for i in range(nf):
                cp_out(i).wait()

    return kernel


def _call(A_x, A_k_cache, A_v_cache, A_wq, A_wo, B_w_gate, B_w_up, B_w_down, c, w_mod,
          G=4, KGA=512, KGB=512, FSQ=256, FC=256, LSQ=256, ffn_mode=0, scopes=False, flags=None):
    x = A_x.reshape(S, D)
    k = A_k_cache.reshape(H, SK, DH)
    v = A_v_cache.reshape(H, SK, DH)
    bf16, f32 = jnp.bfloat16, jnp.float32
    hbm = pl.BlockSpec(memory_space=pl.ANY)
    out = pl.pallas_call(
        _make(G, KGA, KGB, FSQ, FC, LSQ, ffn_mode, scopes),
        in_specs=[pl.BlockSpec(memory_space=pltpu.VMEM)] + [hbm] * 9,
        out_specs=hbm,
        out_shape=jax.ShapeDtypeStruct((S, D), A_x.dtype),
        scratch_shapes=[
            pltpu.VMEM((S, D), bf16),
            pltpu.VMEM((S, D), bf16),
            pltpu.VMEM((H, S, DH), bf16),
            pltpu.VMEM((S, SK), f32),
            pltpu.VMEM((S, 128), f32),
            pltpu.VMEM((SK, DH), bf16),
            pltpu.VMEM((D, DH), bf16),
            pltpu.VMEM((2, G, SK, DH), bf16),
            pltpu.VMEM((2, G, SK, DH), bf16),
            pltpu.VMEM((2, D, G * DH), bf16),
            pltpu.VMEM((H * DH, D), bf16),
            pltpu.VMEM((D, F), bf16),
            pltpu.VMEM((D, F), bf16),
            pltpu.VMEM((F, D), bf16),
            pltpu.VMEM((D, 6 * D), bf16),
            pltpu.VMEM((16, 6 * D), f32),
            pltpu.VMEM((FSQ, D), f32),
            pltpu.VMEM((FSQ, D), bf16),
            pltpu.VMEM((S, D), bf16),
            pltpu.SemaphoreType.DMA((9,)),
            pltpu.SemaphoreType.DMA((2,)),
            pltpu.SemaphoreType.DMA((2,)),
            pltpu.SemaphoreType.DMA((2,)),
            pltpu.SemaphoreType.DMA((S // FSQ,)),
        ],
        compiler_params=pltpu.CompilerParams(vmem_limit_bytes=100 * 1024 * 1024, flags=flags),
    )(c, x, k, v, A_wq, A_wo, B_w_gate, B_w_up, B_w_down, w_mod)
    return out.reshape(1, S, D)


@jax.jit
def pallas_adaLN_cond__mha_block_cached__geglu_ffn__prompt_kernel(
    A_x: jax.Array,
    A_k_cache: jax.Array,
    A_v_cache: jax.Array,
    A_wq: jax.Array,
    A_wo: jax.Array,
    B_x: jax.Array,
    B_w_gate: jax.Array,
    B_w_up: jax.Array,
    B_w_down: jax.Array,
    c: jax.Array,
    w_mod: jax.Array,
):
    del B_x
    return _call(A_x, A_k_cache, A_v_cache, A_wq, A_wo, B_w_gate, B_w_up, B_w_down, c, w_mod, **dict(G=4, flags={"XLA_TPU_FORCE_LP_LLO_SCHEDULER": True}))
```

```python
import math

import jax
import jax.numpy as jnp
from jax import lax
import jax.experimental.pallas as pl
import jax.experimental.pallas.tpu as pltpu

S, D, H, DH, SK, F = 2048, 512, 32, 128, 2048, 1792
NXC = 8
XC = S // NXC
LN_SUB = 8
FB = 256
FC = 256
NF = S // FB
LN2_AFTER = 1
CUT = (0, 1, 5, H - 1)
NG = len(CUT) - 1
QSCALE = (DH ** -0.5) * math.log2(math.e)
_NT = (((1,), (1,)), ((), ()))


def _ln_mod(x, scale1, shift):
    m = jnp.mean(x, axis=-1, keepdims=True)
    xc = x - m
    v = jnp.mean(xc * xc, axis=-1, keepdims=True)
    return xc * lax.rsqrt(v + 1e-5) * scale1 + shift


def _gelu(x):
    return 0.5 * x * (1.0 + jnp.tanh(0.7978845608028654 * (x + 0.044715 * (x * x * x))))


def _lane_tiles(a):
    return [a[:, j * 128:(j + 1) * 128] for j in range(a.shape[-1] // 128)]


def _kernel(c_hbm, x_hbm, k_hbm, v_hbm, wq_hbm, wo_hbm, wg_hbm, wu_hbm, wd_hbm, wmod_hbm, out_hbm,
            c_v, x_v, h_v, acc_v, s_v, m_v, k_v, v_v, wq_v, wo_v, wg_v, wu_v, wd_v, wmod_v, mod_v, out_v,
            sem_misc, sem_x, sem_v, sem_k, sem_q, sem_o, sem_out):
    f32, bf16 = jnp.float32, jnp.bfloat16

    cp_wm0 = pltpu.make_async_copy(wmod_hbm.at[:, pl.ds(0, 2 * D)], wmod_v.at[:, pl.ds(0, 2 * D)], sem_misc.at[0])
    cp_wm1 = pltpu.make_async_copy(wmod_hbm.at[:, pl.ds(2 * D, 4 * D)], wmod_v.at[:, pl.ds(2 * D, 4 * D)],
                                   sem_misc.at[1])
    cp_wg = pltpu.make_async_copy(wg_hbm, wg_v, sem_misc.at[2])
    cp_wu = pltpu.make_async_copy(wu_hbm, wu_v, sem_misc.at[3])
    cp_wd = pltpu.make_async_copy(wd_hbm, wd_v, sem_misc.at[4])
    cp_k0 = pltpu.make_async_copy(k_hbm.at[0], k_v.at[0], sem_misc.at[5])
    cp_q0 = pltpu.make_async_copy(wq_hbm.at[:, pl.ds(0, DH)], wq_v.at[:, pl.ds(0, DH)], sem_misc.at[6])
    cp_c = pltpu.make_async_copy(c_hbm, c_v, sem_misc.at[7])

    def xrows(i):
        return pl.ds(pl.multiple_of(i * XC, XC), XC)

    def cp_x(i):
        return pltpu.make_async_copy(x_hbm.at[xrows(i), :], x_v.at[xrows(i), :], sem_x.at[i])

    def cp_stage(i):
        h0, h1 = CUT[i], CUT[i + 1] + (1 if i == NG - 1 else 0)
        k0, k1 = CUT[i] + 1, CUT[i + 1] + 1
        vs, ks = pl.ds(h0, h1 - h0), pl.ds(k0, k1 - k0)
        qs, os_ = pl.ds(k0 * DH, (k1 - k0) * DH), pl.ds(h0 * DH, (h1 - h0) * DH)
        return (
            pltpu.make_async_copy(v_hbm.at[vs], v_v.at[vs], sem_v.at[i]),
            pltpu.make_async_copy(k_hbm.at[ks], k_v.at[ks], sem_k.at[i]),
            pltpu.make_async_copy(wq_hbm.at[:, qs], wq_v.at[:, qs], sem_q.at[i]),
            pltpu.make_async_copy(wo_hbm.at[os_, :], wo_v.at[os_, :], sem_o.at[i]),
        )

    def start_in_order(steps):
        def issue(i, carry):
            for idx, copies in enumerate(steps):
                @pl.when(i == idx)
                def _():
                    for cp in copies():
                        cp.start()
            return carry
        lax.fori_loop(0, len(steps), issue, 0)

    start_in_order((lambda: (cp_c, cp_wm0), lambda: (cp_q0, cp_x(0)), lambda: (cp_k0, cp_x(1))))
    acc_v[0:S, :] = jnp.zeros((S, D), f32)
    cp_c.wait()
    c = c_v[...].astype(f32)
    sc = jnp.broadcast_to(c * jax.nn.sigmoid(c), (16, D)).astype(bf16)
    cp_wm0.wait()
    for i in range(2, NXC):
        cp_x(i).start()
    mod_v[:, 0:2 * D] = jnp.dot(sc, wmod_v[:, 0:2 * D], preferred_element_type=f32)

    def stage_ln1(i, nsub):
        sa = mod_v[0:1, 0:D]
        ca1 = 1.0 + mod_v[0:1, D:2 * D]
        n = XC // nsub
        for u in range(nsub):
            rows = pl.ds(pl.multiple_of(i * XC + u * n, n), n)
            h_v[rows, :] = _ln_mod(x_v[rows, :].astype(f32), ca1, sa).astype(bf16)

    def stage_q(h, wq):
        q = jnp.dot(h, wq, preferred_element_type=f32)
        return (q * QSCALE).astype(bf16)

    def stage_scores(q, k, rows):
        s = lax.dot_general(q, k, _NT, preferred_element_type=f32)
        s_v[rows, :] = s
        tiles = _lane_tiles(s)
        mx = tiles[0]
        for t in tiles[1:]:
            mx = jnp.maximum(mx, t)
        m_v[rows, :] = mx

    def stage_pv(v):
        m = jnp.broadcast_to(jnp.max(m_v[...], axis=-1, keepdims=True), (S, 128))
        p = jnp.exp2(s_v[...] - jnp.concatenate([m] * (SK // 128), axis=-1))
        tiles = _lane_tiles(p)
        l = tiles[0]
        for t in tiles[1:]:
            l = l + t
        o = jnp.dot(p.astype(bf16), v, preferred_element_type=f32)
        lsum = jnp.sum(l, axis=-1, keepdims=True)
        return (o * pl.reciprocal(lsum, full_range=False)).astype(bf16)

    def stage_out(o, wo):
        acc_v[0:S, :] += jnp.dot(o, wo, preferred_element_type=f32)

    cp_x(0).wait()
    stage_ln1(0, 1)
    cp_q0.wait()
    cp_k0.wait()
    for cp in cp_stage(0):
        cp.start()

    def first_head(i, carry):
        @pl.when(i + 1 < NXC)
        def _():
            cp_x(i + 1).wait()
        q = stage_q(h_v[xrows(i), :], wq_v[:, 0:DH])
        stage_scores(q, k_v[0], xrows(i))
        stage_ln1(jnp.minimum(i + 1, NXC - 1), LN_SUB)
        return carry

    lax.fori_loop(0, NXC, first_head, 0)

    start_in_order((lambda: cp_stage(1), lambda: cp_stage(2)))

    def head_body(hd, carry):
        q = stage_q(h_v[...], wq_v[:, pl.ds(pl.multiple_of((hd + 1) * DH, DH), DH)])
        o = stage_pv(v_v[hd])
        stage_out(o, wo_v[pl.ds(pl.multiple_of(hd * DH, DH), DH), :])
        stage_scores(q, k_v[hd + 1], slice(None))
        return carry

    def stage_body(g, carry):
        lo, hi = CUT[0], CUT[1]
        for i in range(NG):
            @pl.when(g == i)
            def _():
                for cp in cp_stage(i):
                    cp.wait()
                if i == NG - 1:
                    for cp in (cp_wm1, cp_wg, cp_wu, cp_wd):
                        cp.start()
            if i > 0:
                lo = jnp.where(g == i, CUT[i], lo)
                hi = jnp.where(g == i, CUT[i + 1], hi)
        lax.fori_loop(lo, hi, head_body, 0)
        return carry

    lax.fori_loop(0, NG, stage_body, 0)

    cp_wm1.wait()
    cp_wg.wait()
    cp_wu.wait()
    cp_wd.wait()
    mod_v[:, 2 * D:6 * D] = jnp.dot(sc, wmod_v[:, 2 * D:6 * D], preferred_element_type=f32)
    stage_out(stage_pv(v_v[H - 1]), wo_v[(H - 1) * DH:H * DH, :])

    ga = mod_v[0:1, 2 * D:3 * D]
    sb = mod_v[0:1, 3 * D:4 * D]
    cb1 = 1.0 + mod_v[0:1, 4 * D:5 * D]
    gb = mod_v[0:1, 5 * D:6 * D]

    def frows(i):
        if isinstance(i, int):
            return slice(i * FB, (i + 1) * FB)
        return pl.ds(pl.multiple_of(i * FB, FB), FB)

    def cp_out(i):
        rows = pl.ds(pl.multiple_of(i * FB, FB), FB)
        return pltpu.make_async_copy(out_v.at[rows, :], out_hbm.at[rows, :], sem_out.at[i])

    def resid(i):
        return x_v[frows(i), :].astype(f32) + ga * acc_v[frows(i), :]

    def ln2(i):
        return _ln_mod(resid(i), cb1, sb).astype(bf16)

    def store_ln2(i):
        def run():
            h_v[frows(i), :] = ln2(i)
        return run

    def stage_ffn(i, h2, next_ln):
        y = None
        nxt = None
        for f in range(F // FC):
            cols = slice(f * FC, (f + 1) * FC)
            g = jnp.dot(h2, wg_v[:, cols], preferred_element_type=f32)
            u = jnp.dot(h2, wu_v[:, cols], preferred_element_type=f32)
            act = (_gelu(g) * u).astype(bf16)
            yy = jnp.dot(act, wd_v[cols, :], preferred_element_type=f32)
            if f == LN2_AFTER:
                acc_v[pl.ds(pl.multiple_of(S + 8 * (i >> 10), 8), 8), 0:128] = yy[0:8, 0:128]
                nxt = next_ln()
            y = yy if y is None else y + yy
        out_v[frows(i), :] = (resid(i) + gb * y).astype(out_v.dtype)
        cp_out(i).start()
        return nxt

    store_ln2(0)()

    def ffn_body(j, carry):
        i = 2 * j
        h2b = stage_ffn(i, h_v[frows(i), :], lambda: ln2(i + 1))
        stage_ffn(i + 1, h2b, store_ln2(jnp.minimum(i + 2, NF - 1)))
        return carry

    lax.fori_loop(0, NF // 2, ffn_body, 0)
    for i in range(NF):
        cp_out(i).wait()


@jax.jit
def pallas_adaLN_cond__mha_block_cached__geglu_ffn__prompt_kernel(
    A_x: jax.Array,
    A_k_cache: jax.Array,
    A_v_cache: jax.Array,
    A_wq: jax.Array,
    A_wo: jax.Array,
    B_x: jax.Array,
    B_w_gate: jax.Array,
    B_w_up: jax.Array,
    B_w_down: jax.Array,
    c: jax.Array,
    w_mod: jax.Array,
):
    del B_x
    assert A_x.shape == (1, S, D) and A_k_cache.shape == (1, H, SK, DH) and B_w_gate.shape == (D, F)
    bf16, f32 = jnp.bfloat16, jnp.float32
    hbm = pl.BlockSpec(memory_space=pl.ANY)
    dma = pltpu.SemaphoreType.DMA
    out = pl.pallas_call(
        _kernel,
        in_specs=[hbm] * 10,
        out_specs=hbm,
        out_shape=jax.ShapeDtypeStruct((S, D), A_x.dtype),
        scratch_shapes=[
            pltpu.VMEM((1, D), bf16),
            pltpu.VMEM((S, D), bf16),
            pltpu.VMEM((S, D), bf16),
            pltpu.VMEM((S + 8, D), f32),
            pltpu.VMEM((S, SK), f32),
            pltpu.VMEM((S, 128), f32),
            pltpu.VMEM((H, SK, DH), bf16),
            pltpu.VMEM((H, SK, DH), bf16),
            pltpu.VMEM((D, H * DH + 128), bf16),
            pltpu.VMEM((H * DH, D), bf16),
            pltpu.VMEM((D, F), bf16),
            pltpu.VMEM((D, F), bf16),
            pltpu.VMEM((F, D), bf16),
            pltpu.VMEM((D, 6 * D), bf16),
            pltpu.VMEM((16, 6 * D), f32),
            pltpu.VMEM((S, D), bf16),
            dma((8,)), dma((NXC,)), dma((NG,)), dma((NG,)), dma((NG,)), dma((NG,)), dma((NF,)),
        ],
        compiler_params=pltpu.CompilerParams(
            vmem_limit_bytes=110 * 1024 * 1024,
            flags={"XLA_TPU_FORCE_LP_LLO_SCHEDULER": True},
        ),
    )(c, A_x.reshape(S, D), A_k_cache.reshape(H, SK, DH), A_v_cache.reshape(H, SK, DH),
      A_wq, A_wo, B_w_gate, B_w_up, B_w_down, w_mod)
    return out.reshape(1, S, D)
```

```python
import math

import jax
import jax.numpy as jnp
from jax import lax
import jax.experimental.pallas as pl
import jax.experimental.pallas.tpu as pltpu

S, D, H, DH, SK, F = 2048, 512, 32, 128, 2048, 1792
NXC = 8
XC = S // NXC
LN_SUB = 8
FB = 256
FC = 256
NF = S // FB
LN2_STEPS = (1, 2, 3, 4)
CUT = (0, 1, 5, H - 1)
NG = len(CUT) - 1
QSCALE = (DH ** -0.5) * math.log2(math.e)
_NT = (((1,), (1,)), ((), ()))


def _ln_mod(x, scale1, shift):
    m = jnp.mean(x, axis=-1, keepdims=True)
    xc = x - m
    v = jnp.mean(xc * xc, axis=-1, keepdims=True)
    return xc * lax.rsqrt(v + 1e-5) * scale1 + shift


def _gelu(x):
    k = math.sqrt(2.0 / math.pi)
    return 0.5 * x * (1.0 + jnp.tanh(x * (k + (k * 0.044715) * (x * x))))


def _lane_tiles(a):
    return [a[:, j * 128:(j + 1) * 128] for j in range(a.shape[-1] // 128)]


def _kernel(c_hbm, x_hbm, k_hbm, v_hbm, wq_hbm, wo_hbm, wg_hbm, wu_hbm, wd_hbm, wmod_hbm, out_hbm,
            c_v, x_v, h_v, acc_v, s_v, m_v, k_v, v_v, wq_v, wo_v, wg_v, wu_v, wd_v, wmod_v, mod_v, out_v,
            sem_misc, sem_x, sem_v, sem_k, sem_q, sem_o, sem_out):
    f32, bf16 = jnp.float32, jnp.bfloat16

    cp_wm0 = pltpu.make_async_copy(wmod_hbm.at[:, pl.ds(0, 2 * D)], wmod_v.at[:, pl.ds(0, 2 * D)], sem_misc.at[0])
    cp_wm1 = pltpu.make_async_copy(wmod_hbm.at[:, pl.ds(2 * D, 4 * D)], wmod_v.at[:, pl.ds(2 * D, 4 * D)],
                                   sem_misc.at[1])
    cp_wg = pltpu.make_async_copy(wg_hbm, wg_v, sem_misc.at[2])
    cp_wu = pltpu.make_async_copy(wu_hbm, wu_v, sem_misc.at[3])
    cp_wd = pltpu.make_async_copy(wd_hbm, wd_v, sem_misc.at[4])
    cp_k0 = pltpu.make_async_copy(k_hbm.at[0], k_v.at[0], sem_misc.at[5])
    cp_q0 = pltpu.make_async_copy(wq_hbm.at[:, pl.ds(0, DH)], wq_v.at[:, pl.ds(0, DH)], sem_misc.at[6])
    cp_c = pltpu.make_async_copy(c_hbm, c_v, sem_misc.at[7])

    def xrows(i):
        return pl.ds(pl.multiple_of(i * XC, XC), XC)

    def cp_x(i):
        return pltpu.make_async_copy(x_hbm.at[xrows(i), :], x_v.at[xrows(i), :], sem_x.at[i])

    def cp_stage(i):
        h0, h1 = CUT[i], CUT[i + 1] + (1 if i == NG - 1 else 0)
        k0, k1 = CUT[i] + 1, CUT[i + 1] + 1
        vs, ks = pl.ds(h0, h1 - h0), pl.ds(k0, k1 - k0)
        qs, os_ = pl.ds(k0 * DH, (k1 - k0) * DH), pl.ds(h0 * DH, (h1 - h0) * DH)
        return (
            pltpu.make_async_copy(v_hbm.at[vs], v_v.at[vs], sem_v.at[i]),
            pltpu.make_async_copy(k_hbm.at[ks], k_v.at[ks], sem_k.at[i]),
            pltpu.make_async_copy(wq_hbm.at[:, qs], wq_v.at[:, qs], sem_q.at[i]),
            pltpu.make_async_copy(wo_hbm.at[os_, :], wo_v.at[os_, :], sem_o.at[i]),
        )

    def start_in_order(steps):
        def issue(i, carry):
            for idx, copies in enumerate(steps):
                @pl.when(i == idx)
                def _():
                    for cp in copies():
                        cp.start()
            return carry
        lax.fori_loop(0, len(steps), issue, 0)

    start_in_order((lambda: (cp_c, cp_wm0), lambda: (cp_q0, cp_x(0)), lambda: (cp_k0, cp_x(1))))
    acc_v[0:S, :] = jnp.zeros((S, D), f32)
    cp_c.wait()
    c = c_v[...].astype(f32)
    sc = jnp.broadcast_to(c * jax.nn.sigmoid(c), (16, D)).astype(bf16)
    cp_wm0.wait()
    for i in range(2, NXC):
        cp_x(i).start()
    mod_v[:, 0:2 * D] = jnp.dot(sc, wmod_v[:, 0:2 * D], preferred_element_type=f32)

    def stage_ln1(i, nsub):
        sa = mod_v[0:1, 0:D]
        ca1 = 1.0 + mod_v[0:1, D:2 * D]
        n = XC // nsub
        for u in range(nsub):
            rows = pl.ds(pl.multiple_of(i * XC + u * n, n), n)
            h_v[rows, :] = _ln_mod(x_v[rows, :].astype(f32), ca1, sa).astype(bf16)

    def stage_q(h, wq):
        q = jnp.dot(h, wq, preferred_element_type=f32)
        return (q * QSCALE).astype(bf16)

    def stage_scores(q, k, rows):
        s = lax.dot_general(q, k, _NT, preferred_element_type=f32)
        s_v[rows, :] = s
        tiles = _lane_tiles(s)
        mx = tiles[0]
        for t in tiles[1:]:
            mx = jnp.maximum(mx, t)
        m_v[rows, :] = mx

    def stage_pv(v):
        m = jnp.broadcast_to(jnp.max(m_v[...], axis=-1, keepdims=True), (S, 128))
        p = jnp.exp2(s_v[...] - jnp.concatenate([m] * (SK // 128), axis=-1))
        tiles = _lane_tiles(p)
        l = tiles[0]
        for t in tiles[1:]:
            l = l + t
        o = jnp.dot(p.astype(bf16), v, preferred_element_type=f32)
        lsum = jnp.sum(l, axis=-1, keepdims=True)
        return (o * pl.reciprocal(lsum, full_range=False)).astype(bf16)

    def stage_out(o, wo):
        acc_v[0:S, :] += jnp.dot(o, wo, preferred_element_type=f32)

    cp_x(0).wait()
    stage_ln1(0, 1)
    cp_q0.wait()
    cp_k0.wait()
    for cp in cp_stage(0):
        cp.start()

    def first_head(i, carry):
        @pl.when(i + 1 < NXC)
        def _():
            cp_x(i + 1).wait()
        q = stage_q(h_v[xrows(i), :], wq_v[:, 0:DH])
        stage_scores(q, k_v[0], xrows(i))
        stage_ln1(jnp.minimum(i + 1, NXC - 1), LN_SUB)
        return carry

    lax.fori_loop(0, NXC, first_head, 0)

    start_in_order((lambda: cp_stage(1), lambda: cp_stage(2)))

    def head_body(hd, carry):
        q = stage_q(h_v[...], wq_v[:, pl.ds(pl.multiple_of((hd + 1) * DH, DH), DH)])
        o = stage_pv(v_v[hd])
        stage_out(o, wo_v[pl.ds(pl.multiple_of(hd * DH, DH), DH), :])
        stage_scores(q, k_v[hd + 1], slice(None))
        return carry

    def stage_body(g, carry):
        lo, hi = CUT[0], CUT[1]
        for i in range(NG):
            @pl.when(g == i)
            def _():
                for cp in cp_stage(i):
                    cp.wait()
                if i == NG - 1:
                    for cp in (cp_wm1, cp_wg, cp_wu, cp_wd):
                        cp.start()
            if i > 0:
                lo = jnp.where(g == i, CUT[i], lo)
                hi = jnp.where(g == i, CUT[i + 1], hi)
        lax.fori_loop(lo, hi, head_body, 0)
        return carry

    lax.fori_loop(0, NG, stage_body, 0)

    cp_wm1.wait()
    cp_wg.wait()
    cp_wu.wait()
    cp_wd.wait()
    mod_v[:, 2 * D:6 * D] = jnp.dot(sc, wmod_v[:, 2 * D:6 * D], preferred_element_type=f32)
    stage_out(stage_pv(v_v[H - 1]), wo_v[(H - 1) * DH:H * DH, :])

    ga = mod_v[0:1, 2 * D:3 * D]
    sb = mod_v[0:1, 3 * D:4 * D]
    cb1 = 1.0 + mod_v[0:1, 4 * D:5 * D]
    gb = mod_v[0:1, 5 * D:6 * D]

    def frows(i):
        if isinstance(i, int):
            return slice(i * FB, (i + 1) * FB)
        return pl.ds(pl.multiple_of(i * FB, FB), FB)

    def cp_out(i):
        rows = pl.ds(pl.multiple_of(i * FB, FB), FB)
        return pltpu.make_async_copy(out_v.at[rows, :], out_hbm.at[rows, :], sem_out.at[i])

    def resid(rows):
        return x_v[rows, :].astype(f32) + ga * acc_v[rows, :]

    def piece(i, u):
        n = FB // len(LN2_STEPS)
        if isinstance(i, int):
            return slice(i * FB + u * n, i * FB + (u + 1) * n)
        return pl.ds(pl.multiple_of(i * FB + u * n, n), n)

    def ln2(i, u):
        return _ln_mod(resid(piece(i, u)), cb1, sb).astype(bf16)

    def store_ln2(i):
        def run(u):
            h_v[piece(i, u), :] = ln2(i, u)
        return run

    def stage_ffn(i, h2, next_ln):
        y = None
        nxt = []
        for f in range(F // FC):
            cols = slice(f * FC, (f + 1) * FC)
            g = jnp.dot(h2, wg_v[:, cols], preferred_element_type=f32)
            u = jnp.dot(h2, wu_v[:, cols], preferred_element_type=f32)
            act = (_gelu(g) * u).astype(bf16)
            yy = jnp.dot(act, wd_v[cols, :], preferred_element_type=f32)
            if f in LN2_STEPS:
                acc_v[pl.ds(pl.multiple_of(S + 8 * (i >> 10), 8), 8), 0:128] = yy[0:8, 0:128]
                nxt.append(next_ln(LN2_STEPS.index(f)))
            y = yy if y is None else y + yy
        out_v[frows(i), :] = (resid(frows(i)) + gb * y).astype(out_v.dtype)
        cp_out(i).start()
        return nxt

    for u in range(len(LN2_STEPS)):
        store_ln2(0)(u)

    def ffn_body(j, carry):
        i = 2 * j
        h2b = jnp.concatenate(stage_ffn(i, h_v[frows(i), :], lambda u: ln2(i + 1, u)), axis=0)
        stage_ffn(i + 1, h2b, store_ln2(jnp.minimum(i + 2, NF - 1)))
        return carry

    lax.fori_loop(0, NF // 2, ffn_body, 0)
    for i in range(NF):
        cp_out(i).wait()


@jax.jit
def pallas_adaLN_cond__mha_block_cached__geglu_ffn__prompt_kernel(
    A_x: jax.Array,
    A_k_cache: jax.Array,
    A_v_cache: jax.Array,
    A_wq: jax.Array,
    A_wo: jax.Array,
    B_x: jax.Array,
    B_w_gate: jax.Array,
    B_w_up: jax.Array,
    B_w_down: jax.Array,
    c: jax.Array,
    w_mod: jax.Array,
):
    del B_x
    assert A_x.shape == (1, S, D) and A_k_cache.shape == (1, H, SK, DH) and B_w_gate.shape == (D, F)
    bf16, f32 = jnp.bfloat16, jnp.float32
    hbm = pl.BlockSpec(memory_space=pl.ANY)
    dma = pltpu.SemaphoreType.DMA
    out = pl.pallas_call(
        _kernel,
        in_specs=[hbm] * 10,
        out_specs=hbm,
        out_shape=jax.ShapeDtypeStruct((S, D), A_x.dtype),
        scratch_shapes=[
            pltpu.VMEM((1, D), bf16),
            pltpu.VMEM((S, D), bf16),
            pltpu.VMEM((S, D), bf16),
            pltpu.VMEM((S + 8, D), f32),
            pltpu.VMEM((S, SK), f32),
            pltpu.VMEM((S, 128), f32),
            pltpu.VMEM((H, SK, DH), bf16),
            pltpu.VMEM((H, SK, DH), bf16),
            pltpu.VMEM((D, H * DH + 128), bf16),
            pltpu.VMEM((H * DH, D), bf16),
            pltpu.VMEM((D, F), bf16),
            pltpu.VMEM((D, F), bf16),
            pltpu.VMEM((F, D), bf16),
            pltpu.VMEM((D, 6 * D), bf16),
            pltpu.VMEM((16, 6 * D), f32),
            pltpu.VMEM((S, D), bf16),
            dma((8,)), dma((NXC,)), dma((NG,)), dma((NG,)), dma((NG,)), dma((NG,)), dma((NF,)),
        ],
        compiler_params=pltpu.CompilerParams(
            vmem_limit_bytes=110 * 1024 * 1024,
            flags={"XLA_TPU_FORCE_LP_LLO_SCHEDULER": True, "XLA_TPU_EVENLY_DISTRIBUTE_CRITICAL_NODES": True},
        ),
    )(c, A_x.reshape(S, D), A_k_cache.reshape(H, SK, DH), A_v_cache.reshape(H, SK, DH),
      A_wq, A_wo, B_w_gate, B_w_up, B_w_down, w_mod)
    return out.reshape(1, S, D)
```
